```python
import jax
import jax.numpy as jnp

def _softmax(x, axis=-1):
    return jax.nn.softmax(x, axis=axis)
def _gelu(x):
    return jax.nn.gelu(x, approximate=True)
def _silu(x):
    return jax.nn.silu(x)
def _sigmoid(x):
    return jax.nn.sigmoid(x)
def _layernorm(x, axis=-1, eps=1e-5):
    m = jnp.mean(x, axis=axis, keepdims=True)
    v = jnp.var(x, axis=axis, keepdims=True)
    return (x - m) / jnp.sqrt(v + eps)
def _scatter_add(tgt, idx, src, axis=0):
    return tgt.at[idx].add(src)
def _segment_sum(src, seg, n):
    return jax.ops.segment_sum(src, seg, n)
class _Rng:
    def __init__(self, key):
        self._k = key
    def _next(self):
        self._k, sub = jax.random.split(self._k)
        return sub
    def normal(self, shape):
        return jax.random.normal(self._next(), shape, dtype=jnp.bfloat16)
    def randint(self, lo, hi, shape):
        return jax.random.randint(self._next(), shape, lo, hi, dtype=jnp.int32)
    def uniform(self, shape, lo=0.0, hi=1.0):
        return jax.random.uniform(self._next(), shape, jnp.bfloat16, lo, hi)
    def permutation(self, n):
        return jax.random.permutation(self._next(), n)


kernel_name = 'sequential_preLN__mha_block_cached__moe_arch_mod__decode'

def setup_inputs():
    _rng = _Rng(jax.random.key(int.from_bytes(__import__("os").urandom(4), "little")))
    _w = (lambda a: (lambda t: t.astype(jnp.bfloat16) if jnp.issubdtype(t.dtype, jnp.floating) else t)(jnp.asarray(a)))
    def _A_setup():
        B, Sq, D = 4, 1, 640
        H, Sk, Dh = 32, 8192, 192
        return {
            "x": _w((lambda *s: _rng.normal(s) * 0.05)(B, Sq, D)),
            "k_cache": _w((lambda *s: _rng.normal(s) * 0.05)(B, H, Sk, Dh)),
            "v_cache": _w((lambda *s: _rng.normal(s) * 0.05)(B, H, Sk, Dh)),
            "wq": _w((lambda *s: _rng.normal(s) * 0.05)(D, H * Dh) * (D ** -0.5)),
            "wo": _w((lambda *s: _rng.normal(s) * 0.05)(H * Dh, D) * ((H * Dh) ** -0.5)),
        }
    _A_in = _A_setup()

    def _B_setup():
        B, S, D, F, C = 4, 1, 640, 1536, 1
        return {
            "x": _w((lambda *s: _rng.normal(s) * 0.05)(B, S, D)),
            "w_r": _w((lambda *s: _rng.normal(s) * 0.05)(D)),
            "w_gate": _w((lambda *s: _rng.normal(s) * 0.05)(D, F)),
            "w_up": _w((lambda *s: _rng.normal(s) * 0.05)(D, F)),
            "w_down": _w((lambda *s: _rng.normal(s) * 0.05)(F, D)),
        }
    _B_in = _B_setup()

    return {
        "A_x": _A_in["x"],
        "A_k_cache": _A_in["k_cache"],
        "A_v_cache": _A_in["v_cache"],
        "A_wq": _A_in["wq"],
        "A_wo": _A_in["wo"],
        "B_x": _B_in["x"],
        "B_w_r": _B_in["w_r"],
        "B_w_gate": _B_in["w_gate"],
        "B_w_up": _B_in["w_up"],
        "B_w_down": _B_in["w_down"],
    }

def reference(A_x, A_k_cache, A_v_cache, A_wq, A_wo, B_x, B_w_r, B_w_gate, B_w_up, B_w_down):
    def _A_ref(x, k_cache, v_cache, wq, wo):
        B, Sq, D = x.shape
        H, Dh = 32, 192
        q = (lambda x, *d: x.transpose(*d))((x @ wq).reshape(B, Sq, H, Dh), 0, 2, 1, 3)
        scores = jnp.einsum("bhqd,bhkd->bhqk", q, k_cache) * (Dh ** -0.5)
        p = _softmax(scores, axis=-1)
        o = jnp.einsum("bhqk,bhkd->bhqd", p, v_cache)
        return (lambda x, *d: x.transpose(*d))(o, 0, 2, 1, 3).reshape(B, Sq, H * Dh) @ wo

    def _B_ref(x, w_r, w_gate, w_up, w_down):
        B, S, D = x.shape
        C = 1
        r = x @ w_r
        idx = jnp.argsort(-r, axis=-1)[:, :C]
        idx_e = jnp.repeat(idx.reshape(B, C, 1), D, axis=2)
        x_sel = jnp.take_along_axis(x, idx_e, axis=1)
        g = _silu(x_sel @ w_gate)
        u = x_sel @ w_up
        y = (g * u) @ w_down
        r_sel = _sigmoid(jnp.take_along_axis(r, idx, axis=1))
        y = y * r_sel.reshape(B, C, 1)
        b_off = (jnp.arange(B) * S).reshape(B, 1)
        flat_idx = (idx + b_off).reshape(B * C)
        zero = (x * 0.0).reshape(B * S, D)
        upd = _scatter_add(zero, flat_idx, y.reshape(B * C, D), axis=0)
        return x + upd.reshape(B, S, D)

    x = A_x
    h = x + _A_ref(_layernorm(x, axis=-1), A_k_cache, A_v_cache, A_wq, A_wo)
    h2 = h + _B_ref(_layernorm(h, axis=-1), B_w_r, B_w_gate, B_w_up, B_w_down)
    return h2
```

```python
import jax
import jax.numpy as jnp
from jax import lax
import jax.experimental.pallas as pl
import jax.experimental.pallas.tpu as pltpu

B, D, H, SK, DH, F = 4, 640, 32, 8192, 192, 1536
EPS = 1e-5
NBUF = 4
f32, bf16 = jnp.float32, jnp.bfloat16


def _ln(x):
    m = jnp.mean(x, axis=-1, keepdims=True)
    xc = x - m
    v = jnp.mean(xc * xc, axis=-1, keepdims=True)
    return xc / jnp.sqrt(v + EPS)


def _kernel(x_hbm, k_hbm, v_hbm, wq_hbm, wo_hbm, wr_hbm, wg_hbm, wu_hbm, wd_hbm, o_ref,
            kbuf, vbuf, x_v, wq_v, wo_v, wr_v, wg_v, wu_v, wd_v, q_scr, x8, ksem, vsem, wsem):
    total = B * H

    def bh_of(i):
        return (i % B) * H + i // B

    def kcopy(i, slot):
        return pltpu.make_async_copy(k_hbm.at[bh_of(i)], kbuf.at[slot], ksem.at[slot])

    def vcopy(i, slot):
        return pltpu.make_async_copy(v_hbm.at[bh_of(i)], vbuf.at[slot], vsem.at[slot])

    c_x = pltpu.make_async_copy(x_hbm, x_v, wsem.at[0])
    c_wq = pltpu.make_async_copy(wq_hbm, wq_v, wsem.at[1])
    c_wo = pltpu.make_async_copy(wo_hbm, wo_v, wsem.at[2])
    c_wr = pltpu.make_async_copy(wr_hbm, wr_v, wsem.at[3])
    c_wg = pltpu.make_async_copy(wg_hbm, wg_v, wsem.at[4])
    c_wu = pltpu.make_async_copy(wu_hbm, wu_v, wsem.at[5])
    c_wd = pltpu.make_async_copy(wd_hbm, wd_v, wsem.at[6])
    c_x.start()
    c_wq.start()
    kcopy(0, 0).start()
    c_wr.start()
    c_x.wait()
    x8[...] = jnp.zeros((8, D), f32)
    x8[0:B, :] = x_v[...].astype(f32)
    xf = x8[...]
    lnx = _ln(xf).astype(bf16)
    c_wq.wait()
    vcopy(0, 0).start()
    for s in range(1, NBUF):
        kcopy(s, s).start()
        vcopy(s, s).start()
    c_wo.start()
    q = jnp.dot(lnx, wq_v[...], preferred_element_type=f32)
    q = q.astype(bf16).astype(f32)
    for h in range(H):
        q_scr[h] = q[:, h * DH:(h + 1) * DH]
    c_wo.wait()
    row = lax.broadcasted_iota(jnp.int32, (8, DH), 0)

    def head_body(h, acc):
        qh = q_scr[h].astype(bf16)
        oh = jnp.zeros((8, DH), f32)
        for b in range(B):
            i = h * B + b
            slot = b % NBUF
            kcopy(i, slot).wait()
            s = jnp.dot(qh, kbuf[slot], preferred_element_type=f32) * (DH ** -0.5)

            @pl.when(i + NBUF < total)
            def _():
                kcopy(i + NBUF, slot).start()

            m = jnp.max(s, axis=-1, keepdims=True)
            p = jnp.exp(s - m)
            l = jnp.sum(p, axis=-1, keepdims=True)
            vcopy(i, slot).wait()
            o = lax.dot_general(p.astype(bf16), vbuf[slot], (((1,), (1,)), ((), ())),
                                preferred_element_type=f32)

            @pl.when(i + NBUF < total)
            def _():
                vcopy(i + NBUF, slot).start()

            if b == 0:
                @pl.when(h == H - 2)
                def _():
                    c_wg.start()
                    c_wu.start()
                    c_wd.start()
            oh = jnp.where(row == b, o / l, oh)
        return acc + jnp.dot(oh.astype(bf16), wo_v[h], preferred_element_type=f32)

    attn = lax.fori_loop(0, H, head_body, jnp.zeros((8, D), f32))
    hres = (xf + attn.astype(bf16).astype(f32)).astype(bf16).astype(f32)
    lnh_b = _ln(hres).astype(bf16)
    lnh = lnh_b.astype(f32)
    c_wr.wait()
    r = jnp.sum(lnh * wr_v[...].astype(f32), axis=-1, keepdims=True)
    c_wg.wait()
    g = jnp.dot(lnh_b, wg_v[...], preferred_element_type=f32)
    c_wu.wait()
    u = jnp.dot(lnh_b, wu_v[...], preferred_element_type=f32)
    a = (g * jax.nn.sigmoid(g) * u).astype(bf16)
    c_wd.wait()
    y = jnp.dot(a, wd_v[...], preferred_element_type=f32)
    y = y * jax.nn.sigmoid(r)
    out = hres + (lnh + (lnh * 0.0 + y))
    o_ref[...] = out[0:B, :].astype(bf16)


@jax.jit
def pallas_sequential_preLN__mha_block_cached__moe_arch_mod__decode_kernel(
    A_x: jax.Array,
    A_k_cache: jax.Array,
    A_v_cache: jax.Array,
    A_wq: jax.Array,
    A_wo: jax.Array,
    B_x: jax.Array,
    B_w_r: jax.Array,
    B_w_gate: jax.Array,
    B_w_up: jax.Array,
    B_w_down: jax.Array,
):
    del B_x
    kt = jnp.transpose(A_k_cache, (0, 1, 3, 2)).reshape(B * H, DH, SK)
    vt = jnp.transpose(A_v_cache, (0, 1, 3, 2)).reshape(B * H, DH, SK)
    out = pl.pallas_call(
        _kernel,
        in_specs=[pl.BlockSpec(memory_space=pl.ANY)] * 9,
        out_specs=pl.BlockSpec(memory_space=pltpu.VMEM),
        out_shape=jax.ShapeDtypeStruct((B, D), bf16),
        scratch_shapes=[
            pltpu.VMEM((NBUF, DH, SK), bf16), pltpu.VMEM((NBUF, DH, SK), bf16),
            pltpu.VMEM((B, D), bf16), pltpu.VMEM((D, H * DH), bf16), pltpu.VMEM((H, DH, D), bf16),
            pltpu.VMEM((1, D), bf16), pltpu.VMEM((D, F), bf16), pltpu.VMEM((D, F), bf16),
            pltpu.VMEM((F, D), bf16),
            pltpu.VMEM((H, 8, DH), f32), pltpu.VMEM((8, D), f32),
            pltpu.SemaphoreType.DMA((NBUF,)), pltpu.SemaphoreType.DMA((NBUF,)),
            pltpu.SemaphoreType.DMA((7,)),
        ],
        compiler_params=pltpu.CompilerParams(vmem_limit_bytes=100 * 1024 * 1024),
    )(A_x.reshape(B, D), kt, vt, A_wq, A_wo.reshape(H, DH, D), B_w_r.reshape(1, D),
      B_w_gate, B_w_up, B_w_down)
    return out.reshape(B, 1, D)
```

```python
import jax
import jax.numpy as jnp
from jax import lax
import jax.experimental.pallas as pl
import jax.experimental.pallas.tpu as pltpu

B, D, H, SK, DH, F = 4, 640, 32, 8192, 192, 1536
EPS = 1e-5
ND = 4
FC = F // ND
f32, bf16 = jnp.float32, jnp.bfloat16


def _ln(x):
    m = jnp.mean(x, axis=-1, keepdims=True)
    xc = x - m
    v = jnp.mean(xc * xc, axis=-1, keepdims=True)
    return xc / jnp.sqrt(v + EPS)


def _start_cols(src, dst, sem, rows):
    w = 256

    def body(i, carry):
        for r in range(src.shape[0] // rows):
            for t in range(2):
                sl = (pl.ds(r * rows, rows), pl.ds(pl.multiple_of((2 * i + t) * w, w), w))
                pltpu.make_async_copy(src.at[sl], dst.at[sl], sem).start(priority=t)
        return carry

    lax.fori_loop(0, src.shape[1] // (2 * w), body, 0)


def _start_rows(src, dst, sem, rows):
    def body(i, carry):
        for t in range(2):
            sl = pl.ds(pl.multiple_of((2 * i + t) * rows, rows), rows)
            pltpu.make_async_copy(src.at[sl], dst.at[sl], sem).start(priority=t)
        return carry

    lax.fori_loop(0, src.shape[0] // (2 * rows), body, 0)


def _wait(dst, sem):
    pltpu.make_async_copy(dst, dst, sem).wait()


def _kernel(x_hbm, k_hbm, v_hbm, wq_hbm, wo_hbm, wr_hbm, wg_hbm, wu_hbm, wd_hbm, o_ref,
            kbuf, vbuf, x_v, wq_v, wo_v, wr_v, wg_v, wu_v, wd_v, q_scr, x8,
            ksem, vsem, wsem, dsem):
    def kstart(h, b):
        _start_cols(k_hbm.at[b * H + h], kbuf.at[b], ksem.at[b], DH // 2)

    def vstart(h, b):
        _start_cols(v_hbm.at[b * H + h], vbuf.at[b], vsem.at[b], DH // 2)

    def wd_chunk(ref, j):
        return ref.at[pl.ds(j * FC, FC)]

    c_x = pltpu.make_async_copy(x_hbm, x_v, wsem.at[0])
    c_wr = pltpu.make_async_copy(wr_hbm, wr_v, wsem.at[3])

    _start_cols(wq_hbm, wq_v, wsem.at[1], 160)
    c_x.start()
    c_wr.start()
    kstart(0, 0)
    vstart(0, 0)
    c_x.wait()
    x8[...] = jnp.zeros((8, D), f32)
    x8[0:B, :] = x_v[...].astype(f32)
    xf = x8[...]
    lnx = _ln(xf).astype(bf16)
    _wait(wq_v, wsem.at[1])
    kstart(0, 1)
    q = jnp.dot(lnx, wq_v[...], preferred_element_type=f32)
    q = q.astype(bf16).astype(f32)
    for h in range(H):
        q_scr[h] = q[:, h * DH:(h + 1) * DH]
    vstart(0, 1)
    for b in range(2, B):
        kstart(0, b)
        vstart(0, b)
    _start_rows(wo_hbm, wo_v, wsem.at[2], 96)

    row = lax.broadcasted_iota(jnp.int32, (8, DH), 0)

    def head_body(h, acc):
        qh = q_scr[h].astype(bf16)
        oh = jnp.zeros((8, DH), f32)
        more = h + 1 < H
        last = h == H - 1
        for b in range(B):
            _wait(kbuf.at[b], ksem.at[b])
            s = jnp.dot(qh, kbuf[b], preferred_element_type=f32) * (DH ** -0.5)
            pl.when(more)(lambda: kstart(h + 1, b))
            if b == 0:
                pl.when(last)(lambda: _start_cols(wg_hbm, wg_v, wsem.at[4], 160))
            if b == 1:
                @pl.when(last)
                def _():
                    for j in range(ND):
                        _start_rows(wd_chunk(wd_hbm, j), wd_chunk(wd_v, j), dsem.at[j], 96)
            m = jnp.max(s, axis=-1, keepdims=True)
            p = jnp.exp(s - m)
            l = jnp.sum(p, axis=-1, keepdims=True)
            _wait(vbuf.at[b], vsem.at[b])
            o = lax.dot_general(p.astype(bf16), vbuf[b], (((1,), (1,)), ((), ())),
                                preferred_element_type=f32)
            pl.when(more)(lambda: vstart(h + 1, b))
            if b == 0:
                pl.when(last)(lambda: _start_cols(wu_hbm, wu_v, wsem.at[5], 160))
            oh = jnp.where(row == b, o / l, oh)
        pl.when(h == 0)(lambda: _wait(wo_v, wsem.at[2]))
        r0 = pl.multiple_of(h * DH, DH)
        return acc + jnp.dot(oh.astype(bf16), wo_v[pl.ds(r0, DH), :], preferred_element_type=f32)

    attn = lax.fori_loop(0, H, head_body, jnp.zeros((8, D), f32))

    hres = (xf + attn.astype(bf16).astype(f32)).astype(bf16).astype(f32)
    lnh_b = _ln(hres).astype(bf16)
    lnh = lnh_b.astype(f32)
    c_wr.wait()
    wr = wr_v[...].astype(f32)
    rr = lnh[:, 0:128] * wr[0:1, :]
    for j in range(1, D // 128):
        rr = rr + lnh[:, j * 128:(j + 1) * 128] * wr[j:j + 1, :]
    gate = jax.nn.sigmoid(jnp.sum(rr, axis=-1, keepdims=True))
    base = hres + (lnh + lnh * 0.0)
    _wait(wg_v, wsem.at[4])
    g = jnp.dot(lnh_b, wg_v[...], preferred_element_type=f32)
    g = g * jax.nn.sigmoid(g)
    _wait(wu_v, wsem.at[5])
    u = jnp.dot(lnh_b, wu_v[...], preferred_element_type=f32)
    a = (g * u).astype(bf16)
    y = jnp.zeros((8, D), f32)
    for j in range(ND):
        _wait(wd_chunk(wd_v, j), dsem.at[j])
        y = y + jnp.dot(a[:, j * FC:(j + 1) * FC], wd_v[j * FC:(j + 1) * FC, :],
                        preferred_element_type=f32)
    out = base + y * gate
    o_ref[...] = out[0:B, :].astype(bf16)


@jax.jit
def pallas_sequential_preLN__mha_block_cached__moe_arch_mod__decode_kernel(
    A_x: jax.Array,
    A_k_cache: jax.Array,
    A_v_cache: jax.Array,
    A_wq: jax.Array,
    A_wo: jax.Array,
    B_x: jax.Array,
    B_w_r: jax.Array,
    B_w_gate: jax.Array,
    B_w_up: jax.Array,
    B_w_down: jax.Array,
):
    del B_x
    kt = jnp.transpose(A_k_cache, (0, 1, 3, 2)).reshape(B * H, DH, SK)
    vt = jnp.transpose(A_v_cache, (0, 1, 3, 2)).reshape(B * H, DH, SK)
    out = pl.pallas_call(
        _kernel,
        in_specs=[pl.BlockSpec(memory_space=pl.ANY)] * 9,
        out_specs=pl.BlockSpec(memory_space=pltpu.VMEM),
        out_shape=jax.ShapeDtypeStruct((B, D), bf16),
        scratch_shapes=[
            pltpu.VMEM((B, DH, SK), bf16),
            pltpu.VMEM((B, DH, SK), bf16),
            pltpu.VMEM((B, D), bf16),
            pltpu.VMEM((D, H * DH), bf16),
            pltpu.VMEM((H * DH, D), bf16),
            pltpu.VMEM((D // 128, 128), bf16),
            pltpu.VMEM((D, F), bf16),
            pltpu.VMEM((D, F), bf16),
            pltpu.VMEM((F, D), bf16),
            pltpu.VMEM((H, 8, DH), f32),
            pltpu.VMEM((8, D), f32),
            pltpu.SemaphoreType.DMA((B,)),
            pltpu.SemaphoreType.DMA((B,)),
            pltpu.SemaphoreType.DMA((6,)),
            pltpu.SemaphoreType.DMA((ND,)),
        ],
        compiler_params=pltpu.CompilerParams(vmem_limit_bytes=100 * 1024 * 1024),
    )(A_x.reshape(B, D), kt, vt, A_wq, A_wo, B_w_r.reshape(D // 128, 128),
      B_w_gate, B_w_up, B_w_down)
    return out.reshape(B, 1, D)
```

```python
import jax
import jax.numpy as jnp
from jax import lax
import jax.experimental.pallas as pl
import jax.experimental.pallas.tpu as pltpu

B, D, H, SK, DH, F = 4, 640, 32, 8192, 192, 1536
EPS = 1e-5
ND = 4
FC = F // ND
KV_ROWS = (176, 16)
W_ROWS = (160,) * 4
f32, bf16 = jnp.float32, jnp.bfloat16


def _ln(x):
    m = jnp.mean(x, axis=-1, keepdims=True)
    xc = x - m
    v = jnp.mean(xc * xc, axis=-1, keepdims=True)
    return xc / jnp.sqrt(v + EPS)


def _start_cols(src, dst, sem, rows):
    w = 256
    assert sum(rows) == src.shape[0] and src.shape[1] % (2 * w) == 0

    def body(i, carry):
        for j, n in enumerate(rows):
            for t in range(2):
                sl = (pl.ds(sum(rows[:j]), n), pl.ds(pl.multiple_of((2 * i + t) * w, w), w))
                pltpu.make_async_copy(src.at[sl], dst.at[sl], sem).start(priority=t)
        return carry

    lax.fori_loop(0, src.shape[1] // (2 * w), body, 0)


def _start_rows(src, dst, sem, rows):
    assert src.shape[0] % (2 * rows) == 0

    def body(i, carry):
        for t in range(2):
            sl = pl.ds(pl.multiple_of((2 * i + t) * rows, rows), rows)
            pltpu.make_async_copy(src.at[sl], dst.at[sl], sem).start(priority=t)
        return carry

    lax.fori_loop(0, src.shape[0] // (2 * rows), body, 0)


def _wait(dst, sem):
    pltpu.make_async_copy(dst, dst, sem).wait()


def _kernel(x_hbm, k_hbm, v_hbm, wq_hbm, wo_hbm, wr_hbm, wg_hbm, wu_hbm, wd_hbm, o_ref,
            kbuf, vbuf, x_v, wq_v, wo_v, wr_v, wg_v, wu_v, wd_v, q_scr, x8,
            ksem, vsem, wsem, dsem):
    def kstart(h, b):
        _start_cols(k_hbm.at[b * H + h], kbuf.at[b], ksem.at[b], KV_ROWS)

    def vstart(h, b):
        _start_cols(v_hbm.at[b * H + h], vbuf.at[b], vsem.at[b], KV_ROWS)

    def wd_chunk(ref, j):
        return ref.at[pl.ds(j * FC, FC)]

    c_x = pltpu.make_async_copy(x_hbm, x_v, wsem.at[0])
    c_wr = pltpu.make_async_copy(wr_hbm, wr_v, wsem.at[3])

    _start_cols(wq_hbm, wq_v, wsem.at[1], W_ROWS)
    c_x.start()
    c_wr.start()
    kstart(0, 0)
    vstart(0, 0)
    c_x.wait()
    x8[...] = jnp.zeros((8, D), f32)
    x8[0:B, :] = x_v[...].astype(f32)
    xf = x8[...]
    lnx = _ln(xf).astype(bf16)
    _wait(wq_v, wsem.at[1])
    kstart(0, 1)
    q = jnp.dot(lnx, wq_v[...], preferred_element_type=f32)
    q = q.astype(bf16).astype(f32)
    for h in range(H):
        q_scr[h] = q[:, h * DH:(h + 1) * DH]
    vstart(0, 1)
    for b in range(2, B):
        kstart(0, b)
        vstart(0, b)
    _start_rows(wo_hbm, wo_v, wsem.at[2], 96)

    row = lax.broadcasted_iota(jnp.int32, (8, DH), 0)

    def head_body(h, acc):
        qh = q_scr[h].astype(bf16)
        oh = jnp.zeros((8, DH), f32)
        more = h + 1 < H
        last = h == H - 1
        for b in range(B):
            _wait(kbuf.at[b], ksem.at[b])
            s = jnp.dot(qh, kbuf[b], preferred_element_type=f32) * (DH ** -0.5)
            pl.when(more)(lambda: kstart(h + 1, b))
            if b == 0:
                pl.when(last)(lambda: _start_cols(wg_hbm, wg_v, wsem.at[4], W_ROWS))
            if b == 1:
                @pl.when(last)
                def _():
                    for j in range(ND):
                        _start_rows(wd_chunk(wd_hbm, j), wd_chunk(wd_v, j), dsem.at[j], 96)
            m = jnp.max(s, axis=-1, keepdims=True)
            p = jnp.exp(s - m)
            l = jnp.sum(p, axis=-1, keepdims=True)
            _wait(vbuf.at[b], vsem.at[b])
            o = lax.dot_general(p.astype(bf16), vbuf[b], (((1,), (1,)), ((), ())),
                                preferred_element_type=f32)
            pl.when(more)(lambda: vstart(h + 1, b))
            if b == 0:
                pl.when(last)(lambda: _start_cols(wu_hbm, wu_v, wsem.at[5], W_ROWS))
            oh = jnp.where(row == b, o / l, oh)
        pl.when(h == 0)(lambda: _wait(wo_v, wsem.at[2]))
        r0 = pl.multiple_of(h * DH, DH)
        return acc + jnp.dot(oh.astype(bf16), wo_v[pl.ds(r0, DH), :], preferred_element_type=f32)

    attn = lax.fori_loop(0, H, head_body, jnp.zeros((8, D), f32))

    hres = (xf + attn.astype(bf16).astype(f32)).astype(bf16).astype(f32)
    lnh_b = _ln(hres).astype(bf16)
    lnh = lnh_b.astype(f32)
    c_wr.wait()
    wr = wr_v[...].astype(f32)
    rr = lnh[:, 0:128] * wr[0:1, :]
    for j in range(1, D // 128):
        rr = rr + lnh[:, j * 128:(j + 1) * 128] * wr[j:j + 1, :]
    gate = jax.nn.sigmoid(jnp.sum(rr, axis=-1, keepdims=True))
    base = hres + (lnh + lnh * 0.0)
    _wait(wg_v, wsem.at[4])
    g = jnp.dot(lnh_b, wg_v[...], preferred_element_type=f32)
    g = g * jax.nn.sigmoid(g)
    _wait(wu_v, wsem.at[5])
    u = jnp.dot(lnh_b, wu_v[...], preferred_element_type=f32)
    a = (g * u).astype(bf16)
    y = jnp.zeros((8, D), f32)
    for j in range(ND):
        _wait(wd_chunk(wd_v, j), dsem.at[j])
        y = y + jnp.dot(a[:, j * FC:(j + 1) * FC], wd_v[j * FC:(j + 1) * FC, :],
                        preferred_element_type=f32)
    out = base + y * gate
    o_ref[...] = out[0:B, :].astype(bf16)


@jax.jit
def pallas_sequential_preLN__mha_block_cached__moe_arch_mod__decode_kernel(
    A_x: jax.Array,
    A_k_cache: jax.Array,
    A_v_cache: jax.Array,
    A_wq: jax.Array,
    A_wo: jax.Array,
    B_x: jax.Array,
    B_w_r: jax.Array,
    B_w_gate: jax.Array,
    B_w_up: jax.Array,
    B_w_down: jax.Array,
):
    del B_x
    kt = jnp.transpose(A_k_cache, (0, 1, 3, 2)).reshape(B * H, DH, SK)
    vt = jnp.transpose(A_v_cache, (0, 1, 3, 2)).reshape(B * H, DH, SK)
    out = pl.pallas_call(
        _kernel,
        in_specs=[pl.BlockSpec(memory_space=pl.ANY)] * 9,
        out_specs=pl.BlockSpec(memory_space=pltpu.VMEM),
        out_shape=jax.ShapeDtypeStruct((B, D), bf16),
        scratch_shapes=[
            pltpu.VMEM((B, DH, SK), bf16),
            pltpu.VMEM((B, DH, SK), bf16),
            pltpu.VMEM((B, D), bf16),
            pltpu.VMEM((D, H * DH), bf16),
            pltpu.VMEM((H * DH, D), bf16),
            pltpu.VMEM((D // 128, 128), bf16),
            pltpu.VMEM((D, F), bf16),
            pltpu.VMEM((D, F), bf16),
            pltpu.VMEM((F, D), bf16),
            pltpu.VMEM((H, 8, DH), f32),
            pltpu.VMEM((8, D), f32),
            pltpu.SemaphoreType.DMA((B,)),
            pltpu.SemaphoreType.DMA((B,)),
            pltpu.SemaphoreType.DMA((6,)),
            pltpu.SemaphoreType.DMA((ND,)),
        ],
        compiler_params=pltpu.CompilerParams(vmem_limit_bytes=100 * 1024 * 1024),
    )(A_x.reshape(B, D), kt, vt, A_wq, A_wo, B_w_r.reshape(D // 128, 128),
      B_w_gate, B_w_up, B_w_down)
    return out.reshape(B, 1, D)
```
